```python
import jax
import jax.numpy as jnp

def _softmax(x, axis=-1):
    return jax.nn.softmax(x, axis=axis)

def _gelu(x):
    return jax.nn.gelu(x, approximate=True)

def _silu(x):
    return jax.nn.silu(x)

def _sigmoid(x):
    return jax.nn.sigmoid(x)

def _layernorm(x, axis=-1, eps=1e-05):
    m = jnp.mean(x, axis=axis, keepdims=True)
    v = jnp.var(x, axis=axis, keepdims=True)
    return (x - m) / jnp.sqrt(v + eps)

def _scatter_add(tgt, idx, src, axis=0):
    return tgt.at[idx].add(src)

def _segment_sum(src, seg, n):
    return jax.ops.segment_sum(src, seg, n)

class _Rng:

    def __init__(self, key):
        self._k = key

    def _next(self):
        self._k, sub = jax.random.split(self._k)
        return sub

    def normal(self, shape):
        return jax.random.normal(self._next(), shape, dtype=jnp.bfloat16)

    def randint(self, lo, hi, shape):
        return jax.random.randint(self._next(), shape, lo, hi, dtype=jnp.int32)

    def uniform(self, shape, lo=0.0, hi=1.0):
        return jax.random.uniform(self._next(), shape, jnp.bfloat16, lo, hi)

    def permutation(self, n):
        return jax.random.permutation(self._next(), n)
kernel_name = 'adaLN_cond__sliding_block_cached__mixer_gmlp__decode'

def setup_inputs():
    _rng = _Rng(jax.random.key(int.from_bytes(__import__("os").urandom(4), "little")))
    _w = lambda a: (lambda t: t.astype(jnp.bfloat16) if jnp.issubdtype(t.dtype, jnp.floating) else t)(jnp.asarray(a))

    def _A_setup():
        B, Sq, D = (1, 1, 448)
        Hq, Hkv, Sk, Dh = (16, 8, 65536, 256)
        assert Hq % Hkv == 0, (Hq, Hkv)
        return {'x': _w((lambda *s: _rng.normal(s) * 0.05)(B, Sq, D)), 'k_cache': _w((lambda *s: _rng.normal(s) * 0.05)(B, Hkv, Sk, Dh)), 'v_cache': _w((lambda *s: _rng.normal(s) * 0.05)(B, Hkv, Sk, Dh)), 'wq': _w((lambda *s: _rng.normal(s) * 0.05)(D, Hq * Dh) * D ** (-0.5)), 'wo': _w((lambda *s: _rng.normal(s) * 0.05)(Hq * Dh, D) * (Hq * Dh) ** (-0.5))}
    _A_in = _A_setup()

    def _B_setup():
        B, S, D, F = (1, 1, 448, 1792)
        Fh = F // 2
        return {'x': _w((lambda *s: _rng.normal(s) * 0.05)(B, S, D)), 'w_in': _w((lambda *s: _rng.normal(s) * 0.05)(D, 2 * Fh)), 'w_sp': _w(0.01 * (lambda *s: _rng.normal(s) * 0.05)(S, S)), 'b_sp': _w(1.0 + 0.01 * (lambda *s: _rng.normal(s) * 0.05)(S)), 'w_out': _w((lambda *s: _rng.normal(s) * 0.05)(Fh, D))}
    _B_in = _B_setup()
    return {'A_x': _A_in['x'], 'A_k_cache': _A_in['k_cache'], 'A_v_cache': _A_in['v_cache'], 'A_wq': _A_in['wq'], 'A_wo': _A_in['wo'], 'B_x': _B_in['x'], 'B_w_in': _B_in['w_in'], 'B_w_sp': _B_in['w_sp'], 'B_b_sp': _B_in['b_sp'], 'B_w_out': _B_in['w_out'], 'c': _w((lambda *s: _rng.normal(s) * 0.05)(1, 448)), 'w_mod': _w((lambda *s: _rng.normal(s) * 0.05)(448, 6 * 448) * 448 ** (-0.5))}

def reference(A_x, A_k_cache, A_v_cache, A_wq, A_wo, B_x, B_w_in, B_w_sp, B_b_sp, B_w_out, c, w_mod):

    def _A_ref(x, k_cache, v_cache, wq, wo):
        B, Sq, D = x.shape
        Hq, Dh = (16, 256)
        Hkv, Sk = (k_cache.shape[1], k_cache.shape[2])
        W = min(4096, max(256, Sk // 4))
        rep = Hq // Hkv
        q = (lambda x, *d: x.transpose(*d))((x @ wq).reshape(B, Sq, Hq, Dh), 0, 2, 1, 3)
        k = jnp.repeat(k_cache[:, :, Sk - W:, :], rep, axis=1)
        v = jnp.repeat(v_cache[:, :, Sk - W:, :], rep, axis=1)
        scores = jnp.einsum('bhqd,bhkd->bhqk', q, k) * Dh ** (-0.5)
        p = _softmax(scores, axis=-1)
        o = jnp.einsum('bhqk,bhkd->bhqd', p, v)
        return (lambda x, *d: x.transpose(*d))(o, 0, 2, 1, 3).reshape(B, Sq, Hq * Dh) @ wo

    def _B_ref(x, w_in, w_sp, b_sp, w_out):
        B, S, D = x.shape
        F = w_in.shape[-1]
        Fh = F // 2
        z = _gelu(jnp.einsum('bsd,df->bsf', x, w_in))
        z1 = z[..., :Fh].copy()
        z2 = _layernorm(z[..., Fh:], axis=-1)
        g = jnp.einsum('ts,bsf->btf', w_sp, z2) + b_sp[None, :, None]
        return jnp.einsum('bsf,fd->bsd', z1 * g, w_out)
    x = A_x
    mod = (_silu(c) @ w_mod).reshape(c.shape[0], 6, 1, -1)
    sa, ca, ga, sb, cb, gb = (mod[:, 0].copy(), mod[:, 1].copy(), mod[:, 2].copy(), mod[:, 3].copy(), mod[:, 4].copy(), mod[:, 5].copy())
    h = _layernorm(x, axis=-1) * (1 + ca) + sa
    x = x + ga * _A_ref(h, A_k_cache, A_v_cache, A_wq, A_wo)
    h = _layernorm(x, axis=-1) * (1 + cb) + sb
    x = x + gb * _B_ref(h, B_w_in, B_w_sp, B_b_sp, B_w_out)
    return x
```

```python
import functools

import jax
import jax.numpy as jnp
from jax import lax
import jax.experimental.pallas as pl
import jax.experimental.pallas.tpu as pltpu

HQ, DH = 16, 256
F32 = jnp.float32
BF16 = jnp.bfloat16
NT = (((1,), (1,)), ((), ()))
NN = (((1,), (0,)), ((), ()))


def _dot(a, b, dims=NN):
    return lax.dot_general(a, b, dims, preferred_element_type=F32)


def _ln(x, eps=1e-5):
    m = jnp.mean(x, axis=-1, keepdims=True)
    d = x - m
    v = jnp.mean(d * d, axis=-1, keepdims=True)
    return d * lax.rsqrt(v + eps)


def _kernel(x_ref, c_ref, wsp_ref, bsp_ref,
            k_hbm, v_hbm, wq_hbm, woT_hbm, win_hbm, woutT_hbm, wmod_hbm,
            o_ref,
            kbuf, vbuf, wq_buf, wo_buf, win_buf, wout_buf, wmod_buf, sems,
            *, W, Sk, Hkv, D, Fh, nk, nv, window):
    tasks = []
    idx = {}

    def add(name, src, dst):
        i = len(tasks)
        idx[name] = i
        tasks.append(lambda: pltpu.make_async_copy(src(), dst(), sems.at[i]))

    A = 2 * D
    add('wmod_a', lambda: wmod_hbm.at[:, pl.ds(0, A)], lambda: wmod_buf.at[:, pl.ds(0, A)])
    add('wq', lambda: wq_hbm, lambda: wq_buf)
    ck, cv = W // nk, W // nv
    for h in range(Hkv):
        for j in range(nk):
            add(('k', h, j),
                lambda h=h, j=j: k_hbm.at[0, h, pl.ds(Sk - W + j * ck, ck), :],
                lambda h=h, j=j: kbuf.at[h, pl.ds(j * ck, ck), :])
        for j in range(nv):
            add(('v', h, j),
                lambda h=h, j=j: v_hbm.at[0, h, pl.ds(Sk - W + j * cv, cv), :],
                lambda h=h, j=j: vbuf.at[h, pl.ds(j * cv, cv), :])
        if h == 1:
            add('wo', lambda: woT_hbm, lambda: wo_buf)
        if h == 3:
            add('wmod_b', lambda: wmod_hbm.at[:, pl.ds(A, 6 * D - A)],
                lambda: wmod_buf.at[:, pl.ds(A, 6 * D - A)])
    add('win', lambda: win_hbm, lambda: win_buf)
    add('wout', lambda: woutT_hbm, lambda: wout_buf)

    started = [0]

    def start_upto(n):
        while started[0] < min(n, len(tasks)):
            tasks[started[0]]().start()
            started[0] += 1

    def wait(name):
        i = idx[name]
        start_upto(i + 1 + window)
        tasks[i]().wait()

    start_upto(1 + window)

    x = x_ref[0].astype(F32)
    c = c_ref[...].astype(F32)
    cact = jax.nn.silu(c).astype(BF16)
    cact8 = jnp.broadcast_to(cact, (8, D))

    wait('wmod_a')
    mod_a = _dot(cact8, wmod_buf[:, pl.ds(0, A)])[0:1]
    sa = mod_a[:, 0:D]
    ca = mod_a[:, D:2 * D]
    h1 = _ln(x) * (1.0 + ca) + sa
    h8 = jnp.broadcast_to(h1.astype(BF16), (8, D))

    wait('wq')
    row = lax.broadcasted_iota(jnp.int32, (8, DH), 0)
    ya = jnp.zeros((8, D), F32)
    yb = jnp.zeros((8, D), F32)
    mod_b = None
    for h in range(Hkv):
        qa = _dot(h8, wq_buf[:, pl.ds(h * 2 * DH, DH)])
        qb = _dot(h8, wq_buf[:, pl.ds(h * 2 * DH + DH, DH)])
        q = jnp.where(row == 0, qa, qb).astype(BF16)
        ss = []
        for j in range(nk):
            wait(('k', h, j))
            ss.append(_dot(q, kbuf[h, pl.ds(j * ck, ck), :], NT))
        s = jnp.concatenate(ss, axis=1) * (DH ** -0.5) if nk > 1 else ss[0] * (DH ** -0.5)
        m = jnp.max(s, axis=-1, keepdims=True)
        p = jnp.exp(s - m)
        l = jnp.sum(p, axis=-1, keepdims=True)
        pb = p.astype(BF16)
        o = jnp.zeros((8, DH), F32)
        for j in range(nv):
            wait(('v', h, j))
            o = o + _dot(pb[:, j * cv:(j + 1) * cv], vbuf[h, pl.ds(j * cv, cv), :])
        ob = (o / l).astype(BF16)
        if h == 0:
            wait('wo')
        ya = ya + _dot(ob, wo_buf[:, pl.ds(h * 2 * DH, DH)], NT)
        yb = yb + _dot(ob, wo_buf[:, pl.ds(h * 2 * DH + DH, DH)], NT)
        if h == 4:
            wait('wmod_b')
            mod_b = _dot(cact8, wmod_buf[:, pl.ds(A, 6 * D - A)])[0:1]

    y = ya[0:1] + yb[1:2]
    ga = mod_b[:, 0:D]
    sb = mod_b[:, D:2 * D]
    cb = mod_b[:, 2 * D:3 * D]
    gb = mod_b[:, 3 * D:4 * D]
    x1 = x + ga * y
    h2 = _ln(x1) * (1.0 + cb) + sb
    h28 = jnp.broadcast_to(h2.astype(BF16), (8, D))
    wait('win')
    z = jax.nn.gelu(_dot(h28, win_buf[...]), approximate=True)
    z1 = z[:, :Fh]
    z2 = _ln(z[:, Fh:])
    wsp = wsp_ref[...].astype(F32)
    bsp = bsp_ref[...].astype(F32)
    g = wsp * z2 + bsp
    u = (z1 * g).astype(BF16)
    wait('wout')
    out = _dot(u, wout_buf[...], NT)[0:1]
    o_ref[0] = (x1 + gb * out).astype(o_ref.dtype)


@jax.jit
def pallas_adaLN_cond__sliding_block_cached__mixer_gmlp__decode_kernel(
    A_x, A_k_cache, A_v_cache, A_wq, A_wo, B_x, B_w_in, B_w_sp, B_b_sp, B_w_out, c, w_mod,
):
    nk, nv, window = 1, 1, 4
    _, _, D = A_x.shape
    _, Hkv, Sk, _ = A_k_cache.shape
    W = min(4096, max(256, Sk // 4))
    Fh = B_w_in.shape[1] // 2
    ntasks = 2 + Hkv * (nk + nv) + 4
    kern = functools.partial(_kernel, W=W, Sk=Sk, Hkv=Hkv, D=D, Fh=Fh, nk=nk, nv=nv, window=window)
    vm = pl.BlockSpec(memory_space=pltpu.VMEM)
    anyspec = pl.BlockSpec(memory_space=pl.ANY)
    return pl.pallas_call(
        kern,
        out_shape=jax.ShapeDtypeStruct(A_x.shape, A_x.dtype),
        in_specs=[vm, vm, vm, vm] + [anyspec] * 7,
        out_specs=vm,
        scratch_shapes=[
            pltpu.VMEM((Hkv, W, DH), BF16),
            pltpu.VMEM((Hkv, W, DH), BF16),
            pltpu.VMEM(A_wq.shape, BF16),
            pltpu.VMEM(A_wo.shape[::-1], BF16),
            pltpu.VMEM(B_w_in.shape, BF16),
            pltpu.VMEM(B_w_out.shape[::-1], BF16),
            pltpu.VMEM(w_mod.shape, BF16),
            pltpu.SemaphoreType.DMA((ntasks,)),
        ],
        compiler_params=pltpu.CompilerParams(vmem_limit_bytes=100 * 1024 * 1024),
    )(A_x, c, B_w_sp, B_b_sp.reshape(1, 1), A_k_cache, A_v_cache, A_wq, A_wo.T, B_w_in, B_w_out.T, w_mod)
```

```python
import functools

import jax
import jax.numpy as jnp
from jax import lax
import jax.experimental.pallas as pl
import jax.experimental.pallas.tpu as pltpu

_HQ, _DH = 16, 256
_ROWS = 8
_NSEM = 3
_NN = (((1,), (0,)), ((), ()))
_NT = (((1,), (1,)), ((), ()))


def _dot(a, b, dims=_NN):
    return lax.dot_general(a, b, dims, preferred_element_type=jnp.float32)


def _layernorm(x, eps=1e-5):
    m = jnp.mean(x, axis=-1, keepdims=True)
    d = x - m
    v = jnp.mean(d * d, axis=-1, keepdims=True)
    return d * lax.rsqrt(v + eps)


def _lane_chunks(n):
    return [(o, min(128, n - o)) for o in range(0, n, 128)]


def _kernel(x_hbm, c_hbm, wsp_ref, bsp_ref,
            k_hbm, v_hbm, wq_hbm, woT_hbm, win_hbm, woutT_hbm, wmod_hbm,
            o_ref,
            x_buf, c_buf, mod_buf, k_buf, v_buf, wq_buf, wo_buf, win_buf,
            wout_buf, wmod_buf, sems,
            *, window, seq_len, wo_after_head):
    f32, bf16 = jnp.float32, jnp.bfloat16
    n_kv, d_model, f_half = k_buf.shape[0], x_buf.shape[-1], wout_buf.shape[1]
    rep_dh = 2 * _DH
    chunks = _lane_chunks(d_model)

    plan = [(c_hbm, c_buf), (x_hbm, x_buf), (wmod_hbm, wmod_buf), (wq_hbm, wq_buf)]
    for h in range(n_kv):
        plan.append((k_hbm.at[0, h, pl.ds(seq_len - window, window), :], k_buf.at[h]))
        plan.append((v_hbm.at[0, h, pl.ds(seq_len - window, window), :], v_buf.at[h]))
        if h == wo_after_head:
            plan.append((woT_hbm, wo_buf))
    for o, n in chunks:
        plan.append((win_hbm.at[pl.ds(o, n), :], win_buf.at[pl.ds(o, n), :]))
    for o, n in chunks:
        plan.append((woutT_hbm.at[pl.ds(o, n), :], wout_buf.at[pl.ds(o, n), :]))

    copies = [pltpu.make_async_copy(s, d, sems.at[i % _NSEM])
              for i, (s, d) in enumerate(plan)]
    for cp in copies[:_NSEM]:
        cp.start()
    waited = [0]

    def wait_next():
        i = waited[0]
        waited[0] += 1
        copies[i].wait()
        if i + _NSEM < len(copies):
            copies[i + _NSEM].start()

    wait_next()
    cact = jax.nn.silu(c_buf[...].astype(f32)).astype(bf16)
    cact = jnp.broadcast_to(cact, (_ROWS, d_model))
    wait_next()
    x = x_buf[0].astype(f32)
    ln_x = _layernorm(x)
    wait_next()
    mod = _dot(cact, wmod_buf[...])[0:1]
    for i in range(2, 6):
        mod_buf[i - 2] = mod[:, i * d_model:(i + 1) * d_model]
    h1 = ln_x * (1.0 + mod[:, d_model:2 * d_model]) + mod[:, 0:d_model]
    h1 = jnp.broadcast_to(h1.astype(bf16), (_ROWS, d_model))

    wait_next()
    row = lax.broadcasted_iota(jnp.int32, (_ROWS, _DH), 0)
    ya = jnp.zeros((_ROWS, d_model), f32)
    yb = jnp.zeros((_ROWS, d_model), f32)
    pending = []
    for h in range(n_kv):
        qa = _dot(h1, wq_buf[:, pl.ds(h * rep_dh, _DH)])
        qb = _dot(h1, wq_buf[:, pl.ds(h * rep_dh + _DH, _DH)])
        q = (jnp.where(row == 0, qa, qb) * (_DH ** -0.5)).astype(bf16)
        wait_next()
        s = _dot(q, k_buf[h], _NT)
        m = jnp.max(s, axis=-1, keepdims=True)
        p = jnp.exp(s - m)
        l = jnp.sum(p, axis=-1, keepdims=True)
        wait_next()
        o = (_dot(p.astype(bf16), v_buf[h]) / l).astype(bf16)
        pending.append((h, o))
        if h == wo_after_head:
            wait_next()
        if h >= wo_after_head:
            for hh, oo in pending:
                ya = ya + _dot(oo, wo_buf[:, pl.ds(hh * rep_dh, _DH)], _NT)
                yb = yb + _dot(oo, wo_buf[:, pl.ds(hh * rep_dh + _DH, _DH)], _NT)
            pending = []

    y = ya[0:1] + yb[1:2]
    x1 = x + mod_buf[0] * y
    h2 = _layernorm(x1) * (1.0 + mod_buf[2]) + mod_buf[1]
    h2 = jnp.broadcast_to(h2.astype(bf16), (_ROWS, d_model))
    z = None
    for o, n in chunks:
        wait_next()
        t = _dot(h2[:, o:o + n], win_buf[pl.ds(o, n), :])
        z = t if z is None else z + t
    z = jax.nn.gelu(z, approximate=True)
    g = wsp_ref[...].astype(f32) * _layernorm(z[:, f_half:]) + bsp_ref[...].astype(f32)
    u = (z[:, :f_half] * g).astype(bf16)
    gb = mod_buf[3]
    for o, n in chunks:
        wait_next()
        y2 = _dot(u, wout_buf[pl.ds(o, n), :], _NT)[0:1]
        o_ref[0, :, pl.ds(o, n)] = (
            x1[:, o:o + n] + gb[:, o:o + n] * y2).astype(o_ref.dtype)


@jax.jit
def pallas_adaLN_cond__sliding_block_cached__mixer_gmlp__decode_kernel(
    A_x: jax.Array,
    A_k_cache: jax.Array,
    A_v_cache: jax.Array,
    A_wq: jax.Array,
    A_wo: jax.Array,
    B_x: jax.Array,
    B_w_in: jax.Array,
    B_w_sp: jax.Array,
    B_b_sp: jax.Array,
    B_w_out: jax.Array,
    c: jax.Array,
    w_mod: jax.Array,
):
    del B_x
    d_model = A_x.shape[-1]
    _, n_kv, seq_len, _ = A_k_cache.shape
    window = min(4096, max(256, seq_len // 4))
    bf16 = jnp.bfloat16

    kernel = functools.partial(
        _kernel, window=window, seq_len=seq_len, wo_after_head=1)
    vmem = pl.BlockSpec(memory_space=pltpu.VMEM)
    hbm = pl.BlockSpec(memory_space=pl.ANY)
    return pl.pallas_call(
        kernel,
        out_shape=jax.ShapeDtypeStruct(A_x.shape, A_x.dtype),
        in_specs=[hbm, hbm, vmem, vmem] + [hbm] * 7,
        out_specs=vmem,
        scratch_shapes=[
            pltpu.VMEM(A_x.shape, bf16),
            pltpu.VMEM(c.shape, bf16),
            pltpu.VMEM((4, 1, d_model), jnp.float32),
            pltpu.VMEM((n_kv, window, _DH), bf16),
            pltpu.VMEM((n_kv, window, _DH), bf16),
            pltpu.VMEM(A_wq.shape, bf16),
            pltpu.VMEM(A_wo.shape[::-1], bf16),
            pltpu.VMEM(B_w_in.shape, bf16),
            pltpu.VMEM(B_w_out.shape[::-1], bf16),
            pltpu.VMEM(w_mod.shape, bf16),
            pltpu.SemaphoreType.DMA((_NSEM,)),
        ],
        compiler_params=pltpu.CompilerParams(vmem_limit_bytes=64 * 1024 * 1024),
    )(A_x, c, B_w_sp, B_b_sp, A_k_cache, A_v_cache, A_wq,
      A_wo.T, B_w_in, B_w_out.T, w_mod)
```

```python
import functools

import jax
import jax.numpy as jnp
from jax import lax
import jax.experimental.pallas as pl
import jax.experimental.pallas.tpu as pltpu

_HQ, _DH = 16, 256
_ROWS = 8
_NN = (((1,), (0,)), ((), ()))
_NT = (((1,), (1,)), ((), ()))


def _dot(a, b, dims=_NN):
    return lax.dot_general(a, b, dims, preferred_element_type=jnp.float32)


def _layernorm(x, eps=1e-5):
    m = jnp.mean(x, axis=-1, keepdims=True)
    d = x - m
    v = jnp.mean(d * d, axis=-1, keepdims=True)
    return d * lax.rsqrt(v + eps)


def _lane_chunks(n):
    return [(o, min(128, n - o)) for o in range(0, n, 128)]


def _num_copies(n_kv, d_model):
    return 5 + 2 * n_kv + 2 * len(_lane_chunks(d_model))


def _kernel(*refs, **params):
    k_buf, x_buf = refs[15], refs[12]
    n = _num_copies(k_buf.shape[0], x_buf.shape[-1])
    pl.run_scoped(functools.partial(_body, *refs, **params),
                  pltpu.SemaphoreType.DMA((n,)))


def _body(x_hbm, c_hbm, wsp_ref, bsp_ref,
          k_hbm, v_hbm, wq_hbm, woT_hbm, win_hbm, woutT_hbm, wmod_hbm,
          o_ref,
          x_buf, c_buf, mod_buf, k_buf, v_buf, wq_buf, wo_buf, win_buf,
          wout_buf, wmod_buf, sems,
          *, window, seq_len, wo_after_head):
    f32, bf16 = jnp.float32, jnp.bfloat16
    n_kv, d_model, f_half = k_buf.shape[0], x_buf.shape[-1], wout_buf.shape[1]
    rep_dh = 2 * _DH
    chunks = _lane_chunks(d_model)

    plan = [(wmod_hbm, wmod_buf), (c_hbm, c_buf), (x_hbm, x_buf), (wq_hbm, wq_buf)]
    for h in range(n_kv):
        plan.append((k_hbm.at[0, h, pl.ds(seq_len - window, window), :], k_buf.at[h]))
        plan.append((v_hbm.at[0, h, pl.ds(seq_len - window, window), :], v_buf.at[h]))
        if h == wo_after_head:
            plan.append((woT_hbm, wo_buf))
    for o, n in chunks:
        plan.append((win_hbm.at[pl.ds(o, n), :], win_buf.at[pl.ds(o, n), :]))
    for o, n in chunks:
        plan.append((woutT_hbm.at[pl.ds(o, n), :], wout_buf.at[pl.ds(o, n), :]))

    copies = [pltpu.make_async_copy(s, d, sems.at[i])
              for i, (s, d) in enumerate(plan)]
    for cp in copies:
        cp.start()
    waiting = iter(copies)

    def wait_next():
        next(waiting).wait()

    wait_next()
    wait_next()
    cact = jax.nn.silu(c_buf[...].astype(f32)).astype(bf16)
    cact = jnp.broadcast_to(cact, (_ROWS, d_model))
    wait_next()
    x = x_buf[0].astype(f32)
    ln_x = _layernorm(x)
    mod = _dot(cact, wmod_buf[...])[0:1]
    for i in range(2, 6):
        mod_buf[i - 2] = mod[:, i * d_model:(i + 1) * d_model]
    h1 = ln_x * (1.0 + mod[:, d_model:2 * d_model]) + mod[:, 0:d_model]
    h1 = jnp.broadcast_to(h1.astype(bf16), (_ROWS, d_model))

    wait_next()
    row = lax.broadcasted_iota(jnp.int32, (_ROWS, _DH), 0)
    ya = jnp.zeros((_ROWS, d_model), f32)
    yb = jnp.zeros((_ROWS, d_model), f32)
    pending = []
    for h in range(n_kv):
        qa = _dot(h1, wq_buf[:, pl.ds(h * rep_dh, _DH)])
        qb = _dot(h1, wq_buf[:, pl.ds(h * rep_dh + _DH, _DH)])
        q = (jnp.where(row == 0, qa, qb) * (_DH ** -0.5)).astype(bf16)
        wait_next()
        s = _dot(q, k_buf[h], _NT)
        m = jnp.max(s, axis=-1, keepdims=True)
        p = jnp.exp(s - m)
        l = jnp.sum(p, axis=-1, keepdims=True)
        wait_next()
        o = (_dot(p.astype(bf16), v_buf[h]) / l).astype(bf16)
        pending.append((h, o))
        if h == wo_after_head:
            wait_next()
        if h >= wo_after_head:
            for hh, oo in pending:
                ya = ya + _dot(oo, wo_buf[:, pl.ds(hh * rep_dh, _DH)], _NT)
                yb = yb + _dot(oo, wo_buf[:, pl.ds(hh * rep_dh + _DH, _DH)], _NT)
            pending = []

    y = ya[0:1] + yb[1:2]
    x1 = x + mod_buf[0] * y
    h2 = _layernorm(x1) * (1.0 + mod_buf[2]) + mod_buf[1]
    h2 = jnp.broadcast_to(h2.astype(bf16), (_ROWS, d_model))
    z = None
    for o, n in chunks:
        wait_next()
        t = _dot(h2[:, o:o + n], win_buf[pl.ds(o, n), :])
        z = t if z is None else z + t
    z = jax.nn.gelu(z, approximate=True)
    g = wsp_ref[...].astype(f32) * _layernorm(z[:, f_half:]) + bsp_ref[...].astype(f32)
    u = (z[:, :f_half] * g).astype(bf16)
    gb = mod_buf[3]
    for o, n in chunks:
        wait_next()
        y2 = _dot(u, wout_buf[pl.ds(o, n), :], _NT)[0:1]
        o_ref[0, :, pl.ds(o, n)] = (
            x1[:, o:o + n] + gb[:, o:o + n] * y2).astype(o_ref.dtype)


@jax.jit
def pallas_adaLN_cond__sliding_block_cached__mixer_gmlp__decode_kernel(
    A_x: jax.Array,
    A_k_cache: jax.Array,
    A_v_cache: jax.Array,
    A_wq: jax.Array,
    A_wo: jax.Array,
    B_x: jax.Array,
    B_w_in: jax.Array,
    B_w_sp: jax.Array,
    B_b_sp: jax.Array,
    B_w_out: jax.Array,
    c: jax.Array,
    w_mod: jax.Array,
):
    del B_x
    d_model = A_x.shape[-1]
    _, n_kv, seq_len, _ = A_k_cache.shape
    window = min(4096, max(256, seq_len // 4))
    bf16 = jnp.bfloat16

    kernel = functools.partial(
        _kernel, window=window, seq_len=seq_len, wo_after_head=1)
    vmem = pl.BlockSpec(memory_space=pltpu.VMEM)
    hbm = pl.BlockSpec(memory_space=pl.ANY)
    return pl.pallas_call(
        kernel,
        out_shape=jax.ShapeDtypeStruct(A_x.shape, A_x.dtype),
        in_specs=[hbm, hbm, vmem, vmem] + [hbm] * 7,
        out_specs=vmem,
        scratch_shapes=[
            pltpu.VMEM(A_x.shape, bf16),
            pltpu.VMEM(c.shape, bf16),
            pltpu.VMEM((4, 1, d_model), jnp.float32),
            pltpu.VMEM((n_kv, window, _DH), bf16),
            pltpu.VMEM((n_kv, window, _DH), bf16),
            pltpu.VMEM(A_wq.shape, bf16),
            pltpu.VMEM(A_wo.shape[::-1], bf16),
            pltpu.VMEM(B_w_in.shape, bf16),
            pltpu.VMEM(B_w_out.shape[::-1], bf16),
            pltpu.VMEM(w_mod.shape, bf16),
        ],
        compiler_params=pltpu.CompilerParams(vmem_limit_bytes=64 * 1024 * 1024),
    )(A_x, c, B_w_sp, B_b_sp, A_k_cache, A_v_cache, A_wq,
      A_wo.T, B_w_in, B_w_out.T, w_mod)
```

```python
import functools

import jax
import jax.numpy as jnp
from jax import lax
import jax.experimental.pallas as pl
import jax.experimental.pallas.tpu as pltpu

_DH = 256
_ROWS = 8
_NN = (((1,), (0,)), ((), ()))
_NT = (((1,), (1,)), ((), ()))


def _dot(a, b, dims=_NN):
    return lax.dot_general(a, b, dims, preferred_element_type=jnp.float32)


def _layernorm(x, eps=1e-5):
    m = jnp.mean(x, axis=-1, keepdims=True)
    d = x - m
    v = jnp.mean(d * d, axis=-1, keepdims=True)
    return d * lax.rsqrt(v + eps)


def _lane_chunks(n):
    return [(o, min(128, n - o)) for o in range(0, n, 128)]


def _kernel(*refs, n_copies, **params):
    pl.run_scoped(functools.partial(_body, *refs, **params),
                  pltpu.SemaphoreType.DMA((n_copies,)))


def _body(x_hbm, c_hbm, wsp_ref, bsp_ref,
          k_hbm, v_hbm, wq_hbm, woT_hbm, win_hbm, woutT_hbm, wmod_hbm,
          o_ref,
          x_buf, c_buf, mod_buf, k_buf, v_buf, wq_buf, wo_buf, win_buf,
          wout_buf, wmod_buf, sems,
          *, window, seq_len):
    f32, bf16 = jnp.float32, jnp.bfloat16
    n_kv, d_model, f_half = k_buf.shape[0], x_buf.shape[-1], wout_buf.shape[1]
    rep_dh = 2 * _DH
    chunks = _lane_chunks(d_model)

    plan = [(wmod_hbm, wmod_buf), (c_hbm, c_buf), (x_hbm, x_buf),
            (wq_hbm, wq_buf), (woT_hbm, wo_buf)]
    for h in range(n_kv):
        plan.append((k_hbm.at[0, h, pl.ds(seq_len - window, window), :], k_buf.at[h]))
        plan.append((v_hbm.at[0, h, pl.ds(seq_len - window, window), :], v_buf.at[h]))
    for o, n in chunks:
        plan.append((win_hbm.at[pl.ds(o, n), :], win_buf.at[pl.ds(o, n), :]))
    for o, n in chunks:
        plan.append((woutT_hbm.at[pl.ds(o, n), :], wout_buf.at[pl.ds(o, n), :]))

    assert len(plan) == sems.shape[0]
    copies = [pltpu.make_async_copy(s, d, sems.at[i])
              for i, (s, d) in enumerate(plan)]
    for cp in copies:
        cp.start()
    waiting = iter(copies)

    def wait_next():
        next(waiting).wait()

    wait_next()
    wait_next()
    cact = jax.nn.silu(c_buf[...].astype(f32)).astype(bf16)
    cact = jnp.broadcast_to(cact, (_ROWS, d_model))
    wait_next()
    x = x_buf[0].astype(f32)
    ln_x = _layernorm(x)
    mod = _dot(cact, wmod_buf[...])[0:1]
    for i in range(2, 6):
        mod_buf[i - 2] = mod[:, i * d_model:(i + 1) * d_model]
    h1 = ln_x * (1.0 + mod[:, d_model:2 * d_model]) + mod[:, 0:d_model]
    h1 = jnp.broadcast_to(h1.astype(bf16), (_ROWS, d_model))

    wait_next()
    wait_next()
    row = lax.broadcasted_iota(jnp.int32, (_ROWS, _DH), 0)
    ya = jnp.zeros((_ROWS, d_model), f32)
    yb = jnp.zeros((_ROWS, d_model), f32)
    for h in range(n_kv):
        qa = _dot(h1, wq_buf[:, pl.ds(h * rep_dh, _DH)])
        qb = _dot(h1, wq_buf[:, pl.ds(h * rep_dh + _DH, _DH)])
        q = (jnp.where(row == 0, qa, qb) * (_DH ** -0.5)).astype(bf16)
        wait_next()
        s = _dot(q, k_buf[h], _NT)
        m = jnp.max(s, axis=-1, keepdims=True)
        p = jnp.exp(s - m)
        l = jnp.sum(p, axis=-1, keepdims=True)
        wait_next()
        o = (_dot(p.astype(bf16), v_buf[h]) / l).astype(bf16)
        ya = ya + _dot(o, wo_buf[:, pl.ds(h * rep_dh, _DH)], _NT)
        yb = yb + _dot(o, wo_buf[:, pl.ds(h * rep_dh + _DH, _DH)], _NT)

    y = ya[0:1] + yb[1:2]
    x1 = x + mod_buf[0] * y
    h2 = _layernorm(x1) * (1.0 + mod_buf[2]) + mod_buf[1]
    h2 = jnp.broadcast_to(h2.astype(bf16), (_ROWS, d_model))
    z = None
    for o, n in chunks:
        wait_next()
        t = _dot(h2[:, o:o + n], win_buf[pl.ds(o, n), :])
        z = t if z is None else z + t
    z = jax.nn.gelu(z, approximate=True)
    g = wsp_ref[...].astype(f32) * _layernorm(z[:, f_half:]) + bsp_ref[...].astype(f32)
    u = (z[:, :f_half] * g).astype(bf16)
    gb = mod_buf[3]
    for o, n in chunks:
        wait_next()
        y2 = _dot(u, wout_buf[pl.ds(o, n), :], _NT)[0:1]
        o_ref[0, :, pl.ds(o, n)] = (
            x1[:, o:o + n] + gb[:, o:o + n] * y2).astype(o_ref.dtype)


@jax.jit
def pallas_adaLN_cond__sliding_block_cached__mixer_gmlp__decode_kernel(
    A_x: jax.Array,
    A_k_cache: jax.Array,
    A_v_cache: jax.Array,
    A_wq: jax.Array,
    A_wo: jax.Array,
    B_x: jax.Array,
    B_w_in: jax.Array,
    B_w_sp: jax.Array,
    B_b_sp: jax.Array,
    B_w_out: jax.Array,
    c: jax.Array,
    w_mod: jax.Array,
):
    del B_x
    d_model = A_x.shape[-1]
    _, n_kv, seq_len, _ = A_k_cache.shape
    window = min(4096, max(256, seq_len // 4))
    bf16 = jnp.bfloat16

    n_copies = 5 + 2 * n_kv + 2 * len(_lane_chunks(d_model))
    kernel = functools.partial(
        _kernel, window=window, seq_len=seq_len, n_copies=n_copies)
    vmem = pl.BlockSpec(memory_space=pltpu.VMEM)
    hbm = pl.BlockSpec(memory_space=pl.ANY)
    return pl.pallas_call(
        kernel,
        out_shape=jax.ShapeDtypeStruct(A_x.shape, A_x.dtype),
        in_specs=[hbm, hbm, vmem, vmem] + [hbm] * 7,
        out_specs=vmem,
        scratch_shapes=[
            pltpu.VMEM(A_x.shape, bf16),
            pltpu.VMEM(c.shape, bf16),
            pltpu.VMEM((4, 1, d_model), jnp.float32),
            pltpu.VMEM((n_kv, window, _DH), bf16),
            pltpu.VMEM((n_kv, window, _DH), bf16),
            pltpu.VMEM(A_wq.shape, bf16),
            pltpu.VMEM(A_wo.shape[::-1], bf16),
            pltpu.VMEM(B_w_in.shape, bf16),
            pltpu.VMEM(B_w_out.shape[::-1], bf16),
            pltpu.VMEM(w_mod.shape, bf16),
        ],
        compiler_params=pltpu.CompilerParams(vmem_limit_bytes=64 * 1024 * 1024),
    )(A_x, c, B_w_sp, B_b_sp, A_k_cache, A_v_cache, A_wq,
      A_wo.T, B_w_in, B_w_out.T, w_mod)
```
